```python
import os as _os
_os.environ.setdefault("JAX_PLATFORMS", "cpu")
import jax
import jax.numpy as jnp

def _softmax(x, axis=-1):
    return jax.nn.softmax(x, axis=axis)
def _gelu(x):
    return jax.nn.gelu(x, approximate=True)
def _silu(x):
    return jax.nn.silu(x)
def _sigmoid(x):
    return jax.nn.sigmoid(x)
def _layernorm(x, axis=-1, eps=1e-5):
    m = jnp.mean(x, axis=axis, keepdims=True)
    v = jnp.var(x, axis=axis, keepdims=True)
    return (x - m) / jnp.sqrt(v + eps)
def _scatter_add(tgt, idx, src, axis=0):
    return tgt.at[idx].add(src)
def _segment_sum(src, seg, n):
    return jax.ops.segment_sum(src, seg, n)
class _Rng:
    def __init__(self, key):
        self._k = key
    def _next(self):
        self._k, sub = jax.random.split(self._k)
        return sub
    def normal(self, shape):
        return jax.random.normal(self._next(), shape, dtype=jnp.bfloat16)
    def randint(self, lo, hi, shape):
        return jax.random.randint(self._next(), shape, lo, hi, dtype=jnp.int32)
    def uniform(self, shape, lo=0.0, hi=1.0):
        return jax.random.uniform(self._next(), shape, jnp.bfloat16, lo, hi)
    def permutation(self, n):
        return jax.random.permutation(self._next(), n)


kernel_name = 'sequential_preLN__compressed_kv_cla__dense_activation_mish__decode'

def setup_inputs():
    _rng = _Rng(jax.random.key(int.from_bytes(__import__("os").urandom(4), "little")))
    _w = (lambda a: (lambda t: t.astype(jnp.bfloat16) if jnp.issubdtype(t.dtype, jnp.floating) else t)(jnp.asarray(a)))
    def _A_setup():
        B, H, Sq, Sk, D, M = 1, 32, 1, 8192, 128, 512
        Dc = 4 * D
        return {
            "x": _w((lambda *s: _rng.normal(s) * 0.05)(B, Sq, M)),
            "c_kv": _w((lambda *s: _rng.normal(s) * 0.8)(B, Sk, Dc)),
            "w_q": _w((lambda *s: _rng.normal(s) * 0.8)(M, H, D) * (M ** -0.5)),
            "w_uk": _w((lambda *s: _rng.normal(s) * 0.8)(Dc, H, D) * (Dc ** -0.5)),
            "w_uv": _w((lambda *s: _rng.normal(s) * 0.8)(Dc, H, D) * (Dc ** -0.5)),
            "w_o": _w((lambda *s: _rng.normal(s) * 0.8)(H, D, M) * ((H * D) ** -0.5)),
        }
    _A_in = _A_setup()

    def _B_setup():
        B, S, D, F = 1, 1, 512, 1376
        return {
            "x": _w((lambda *s: _rng.normal(s) * 0.05)(B, S, D)),
            "w1": _w((lambda *s: _rng.normal(s) * 0.2)(D, F) * (D ** -0.5)),
            "b1": _w((lambda *s: _rng.normal(s) * 0.05)(F)),
            "w2": _w((lambda *s: _rng.normal(s) * 0.05)(F, D) * (F ** -0.5)),
        }
    _B_in = _B_setup()

    return {
        "A_x": _A_in["x"],
        "A_c_kv": _A_in["c_kv"],
        "A_w_q": _A_in["w_q"],
        "A_w_uk": _A_in["w_uk"],
        "A_w_uv": _A_in["w_uv"],
        "A_w_o": _A_in["w_o"],
        "B_x": _B_in["x"],
        "B_w1": _B_in["w1"],
        "B_b1": _B_in["b1"],
        "B_w2": _B_in["w2"],
    }

def reference(A_x, A_c_kv, A_w_q, A_w_uk, A_w_uv, A_w_o, B_x, B_w1, B_b1, B_w2):
    def _A_ref(x, c_kv, w_q, w_uk, w_uv, w_o):
        B, Sq, M = x.shape[0], x.shape[1], x.shape[2]
        Sk = c_kv.shape[1]
        H, D = w_q.shape[1], w_q.shape[2]
        q = jnp.einsum("bqm,mhd->bhqd", x, w_q)
        k = jnp.einsum("bkc,chd->bhkd", c_kv, w_uk)
        v = jnp.einsum("bkc,chd->bhkd", c_kv, w_uv)
        scores = jnp.einsum("bhqd,bhkd->bhqk", q, k) * (D ** -0.5)
        off = Sk - Sq
        qi = jnp.arange(Sq)[:, None]
        kj = jnp.arange(Sk)[None, :]
        cmask = kj <= (qi + off)
        scores = jnp.where(cmask[None, None], scores, -1e9)
        p = _softmax(scores, axis=-1)
        ctx = jnp.einsum("bhqk,bhkd->bhqd", p, v)
        return jnp.einsum("bhqd,hdm->bqm", ctx, w_o)

    def _B_ref(x, w1, b1, w2):
        h = jnp.einsum("bsd,df->bsf", x, w1) + b1
        sp = jnp.log1p(jnp.exp(-jnp.abs(h))) + jnp.where(h > 0, h, jnp.zeros_like(h))
        act = h * jnp.tanh(sp)
        return jnp.einsum("bsf,fd->bsd", act, w2)

    x = A_x
    h = x + _A_ref(_layernorm(x, axis=-1), A_c_kv, A_w_q, A_w_uk, A_w_uv, A_w_o)
    h2 = h + _B_ref(_layernorm(h, axis=-1), B_w1, B_b1, B_w2)
    return h2
```

```python
import functools

import jax
import jax.numpy as jnp
from jax import lax
import jax.experimental.pallas as pl
import jax.experimental.pallas.tpu as pltpu

_EPS = 1e-5
_KV_CHUNKS = 4
_W2_SPLITS = (0, 1024, 1280, 1376)


def _layernorm(x):
    m = jnp.mean(x, axis=-1, keepdims=True)
    d = x - m
    v = jnp.mean(d * d, axis=-1, keepdims=True)
    return d * lax.rsqrt(v + _EPS)


def _nt(a, b):
    return lax.dot_general(a, b, (((1,), (1,)), ((), ())), preferred_element_type=jnp.float32)


def _nn(a, b):
    return jnp.dot(a, b, preferred_element_type=jnp.float32)


def _kernel(x_hbm, ckv_hbm, wq_hbm, wuk_hbm, wuv_hbm, wo_hbm, w1t_hbm, b1_hbm, w2_hbm,
            o_ref,
            x_v, b1_v, wq_v, wuk_v, ckv_v, wuv_v, wo_v, w1t_v, w2_v, sems,
            *, H, D, scale):
    bf16, f32 = jnp.bfloat16, jnp.float32
    Sk, Dc = ckv_v.shape
    M = x_v.shape[-1]
    npair = H // 2
    kc = Sk // _KV_CHUNKS

    copies = []

    def add(src, dst):
        c = pltpu.make_async_copy(src, dst, sems.at[len(copies)])
        copies.append(c)
        return c

    c_x = add(x_hbm, x_v)
    c_b1 = add(b1_hbm, b1_v)
    c_wq = add(wq_hbm, wq_v)
    c_wuk = add(wuk_hbm, wuk_v)
    c_kv = [add(ckv_hbm.at[pl.ds(i * kc, kc)], ckv_v.at[pl.ds(i * kc, kc)])
            for i in range(_KV_CHUNKS)]
    c_wuv = add(wuv_hbm, wuv_v)
    c_wo = add(wo_hbm, wo_v)
    c_w1 = add(w1t_hbm, w1t_v)
    c_w2 = [add(w2_hbm.at[pl.ds(a, b - a)], w2_v.at[pl.ds(a, b - a)])
            for a, b in zip(_W2_SPLITS[:-1], _W2_SPLITS[1:])]
    for c in copies:
        c.start()

    def pair(w_ref, i):
        w32 = w_ref.bitcast(jnp.uint32)
        return pltpu.bitcast(w32[pl.ds(i, Dc, stride=npair), :], bf16)

    er = lax.broadcasted_iota(jnp.int32, (Dc, 2 * Dc), 0)
    ec = lax.broadcasted_iota(jnp.int32, (Dc, 2 * Dc), 1)
    expand = jnp.where(ec // 2 == er, 1.0, 0.0).astype(bf16)
    row2 = lax.broadcasted_iota(jnp.int32, (H, 2 * Dc), 0)
    col2 = lax.broadcasted_iota(jnp.int32, (H, 2 * Dc), 1)
    parity = (row2 % 2) == (col2 % 2)
    pair2 = row2 // 2
    rowd = lax.broadcasted_iota(jnp.int32, (H, D), 0)

    c_x.wait()
    x = x_v[0].astype(f32)
    xn = _layernorm(x).astype(bf16)
    xe = _nn(jnp.broadcast_to(xn, (H, M)), expand)
    xe = jnp.where(parity, xe, 0.0)
    c_wq.wait()
    q = jnp.zeros((H, D), f32)
    for i in range(npair):
        q = q + _nn(jnp.where(pair2 == i, xe, 0.0).astype(bf16), pair(wq_v, i))

    c_wuk.wait()
    s2 = jnp.zeros((H, 2 * Dc), f32)
    for i in range(npair):
        s2 = s2 + _nt(jnp.where(rowd // 2 == i, q, 0.0).astype(bf16), pair(wuk_v, i))
    s2 = jnp.where(parity, s2 * scale, 0.0).astype(bf16)
    q_lat = _nt(s2, expand).astype(bf16)

    m = jnp.full((H, 1), -jnp.inf, f32)
    l = jnp.zeros((H, 1), f32)
    acc = jnp.zeros((H, Dc), f32)
    for i in range(_KV_CHUNKS):
        c_kv[i].wait()
        kv = ckv_v[pl.ds(i * kc, kc), :]
        s = _nt(q_lat, kv)
        m_new = jnp.maximum(m, jnp.max(s, axis=-1, keepdims=True))
        a = jnp.exp(m - m_new)
        p = jnp.exp(s - m_new)
        l = a * l + jnp.sum(p, axis=-1, keepdims=True)
        acc = a * acc + _nn(p.astype(bf16), kv)
        m = m_new
    ctx_lat = (acc / l).astype(bf16)

    ce = jnp.where(parity, _nn(ctx_lat, expand), 0.0)
    c_wuv.wait()
    ctx = jnp.zeros((H, D), f32)
    for i in range(npair):
        ctx = ctx + _nn(jnp.where(pair2 == i, ce, 0.0).astype(bf16), pair(wuv_v, i))

    c_wo.wait()
    ao = jnp.zeros((H, M), f32)
    for h in range(H):
        ao = ao + _nn(jnp.where(rowd == h, ctx, 0.0).astype(bf16), wo_v[pl.ds(h * D, D), :])
    h1 = x + jnp.sum(ao, axis=0, keepdims=True)

    hn = jnp.broadcast_to(_layernorm(h1).astype(bf16), (16, M))
    c_w1.wait()
    c_b1.wait()
    z = _nt(hn, w1t_v[...]) + b1_v[...].astype(f32).reshape(1, -1)
    sp = jnp.log1p(jnp.exp(-jnp.abs(z))) + jnp.where(z > 0, z, 0.0)
    act = (z * jnp.tanh(sp)).astype(bf16)
    out = jnp.broadcast_to(h1, (16, M))
    for j, (a0, b0) in enumerate(zip(_W2_SPLITS[:-1], _W2_SPLITS[1:])):
        c_w2[j].wait()
        out = out + _nn(act[:, a0:b0], w2_v[pl.ds(a0, b0 - a0), :])
    o_ref[0] = out[0:1, :].astype(o_ref.dtype)


@jax.jit
def pallas_sequential_preLN__compressed_kv_cla__dense_activation_mish__decode_kernel(
    A_x: jax.Array,
    A_c_kv: jax.Array,
    A_w_q: jax.Array,
    A_w_uk: jax.Array,
    A_w_uv: jax.Array,
    A_w_o: jax.Array,
    B_x: jax.Array,
    B_w1: jax.Array,
    B_b1: jax.Array,
    B_w2: jax.Array,
):
    del B_x
    M, H, D = A_w_q.shape
    _, Sk, Dc = A_c_kv.shape
    F = B_w1.shape[1]
    dt = A_x.dtype
    any_spec = pl.BlockSpec(memory_space=pl.ANY)
    n_dma = 7 + _KV_CHUNKS + len(_W2_SPLITS) - 1
    return pl.pallas_call(
        functools.partial(_kernel, H=H, D=D, scale=D ** -0.5),
        out_shape=jax.ShapeDtypeStruct(A_x.shape, dt),
        in_specs=[any_spec] * 9,
        out_specs=pl.BlockSpec(memory_space=pltpu.VMEM),
        scratch_shapes=[
            pltpu.VMEM(A_x.shape, dt),
            pltpu.VMEM((F,), dt),
            pltpu.VMEM((M * H, D), dt),
            pltpu.VMEM((Dc * H, D), dt),
            pltpu.VMEM((Sk, Dc), dt),
            pltpu.VMEM((Dc * H, D), dt),
            pltpu.VMEM((H * D, M), dt),
            pltpu.VMEM((F, M), dt),
            pltpu.VMEM((F, M), dt),
            pltpu.SemaphoreType.DMA((n_dma,)),
        ],
        compiler_params=pltpu.CompilerParams(vmem_limit_bytes=64 * 1024 * 1024),
    )(
        A_x,
        A_c_kv.reshape(Sk, Dc),
        A_w_q.reshape(M * H, D),
        A_w_uk.reshape(Dc * H, D),
        A_w_uv.reshape(Dc * H, D),
        A_w_o.reshape(H * D, M),
        B_w1.T,
        B_b1,
        B_w2,
    )
```
